```python
import jax
import jax.numpy as jnp

def _softmax(x, axis=-1):
    return jax.nn.softmax(x, axis=axis)
def _gelu(x):
    return jax.nn.gelu(x, approximate=True)
def _silu(x):
    return jax.nn.silu(x)
def _sigmoid(x):
    return jax.nn.sigmoid(x)
def _layernorm(x, axis=-1, eps=1e-5):
    m = jnp.mean(x, axis=axis, keepdims=True)
    v = jnp.var(x, axis=axis, keepdims=True)
    return (x - m) / jnp.sqrt(v + eps)
def _scatter_add(tgt, idx, src, axis=0):
    return tgt.at[idx].add(src)
def _segment_sum(src, seg, n):
    return jax.ops.segment_sum(src, seg, n)
class _Rng:
    def __init__(self, key):
        self._k = key
    def _next(self):
        self._k, sub = jax.random.split(self._k)
        return sub
    def normal(self, shape):
        return jax.random.normal(self._next(), shape, dtype=jnp.bfloat16)
    def randint(self, lo, hi, shape):
        return jax.random.randint(self._next(), shape, lo, hi, dtype=jnp.int32)
    def uniform(self, shape, lo=0.0, hi=1.0):
        return jax.random.uniform(self._next(), shape, jnp.bfloat16, lo, hi)
    def permutation(self, n):
        return jax.random.permutation(self._next(), n)


kernel_name = 'gated_mix__linear_attn_block__moe_arch_mod__prompt'

def setup_inputs():
    _rng = _Rng(jax.random.key(int.from_bytes(__import__("os").urandom(4), "little")))
    _w = (lambda a: (lambda t: t.astype(jnp.bfloat16) if jnp.issubdtype(t.dtype, jnp.floating) else t)(jnp.asarray(a)))
    def _A_setup():
        B, S, D = 1, 2048, 1024
        return {
            "x": _w((lambda *s: _rng.normal(s) * 0.05)(B, S, D)),
            "wqkv": _w((lambda *s: _rng.normal(s) * 0.05)(D, 3 * D)),
            "wo": _w((lambda *s: _rng.normal(s) * 0.05)(D, D)),
        }
    _A_in = _A_setup()

    def _B_setup():
        B, S, D, F, C = 1, 2048, 1024, 3584, 1
        return {
            "x": _w((lambda *s: _rng.normal(s) * 0.05)(B, S, D)),
            "w_r": _w((lambda *s: _rng.normal(s) * 0.05)(D)),
            "w_gate": _w((lambda *s: _rng.normal(s) * 0.05)(D, F)),
            "w_up": _w((lambda *s: _rng.normal(s) * 0.05)(D, F)),
            "w_down": _w((lambda *s: _rng.normal(s) * 0.05)(F, D)),
        }
    _B_in = _B_setup()

    return {
        "A_x": _A_in["x"],
        "A_wqkv": _A_in["wqkv"],
        "A_wo": _A_in["wo"],
        "B_x": _B_in["x"],
        "B_w_r": _B_in["w_r"],
        "B_w_gate": _B_in["w_gate"],
        "B_w_up": _B_in["w_up"],
        "B_w_down": _B_in["w_down"],
        "gate_w": _w((lambda *s: _rng.normal(s) * 0.05)(1024)),
    }

def reference(A_x, A_wqkv, A_wo, B_x, B_w_r, B_w_gate, B_w_up, B_w_down, gate_w):
    def _A_ref(x, wqkv, wo):
        B, S, D = x.shape
        H = 32; Dh = D // H
        qkv = (lambda x, *d: x.transpose(*d))((x @ wqkv).reshape(B, S, 3, H, Dh), 2, 0, 3, 1, 4)
        q, k, v = qkv[0], qkv[1], qkv[2]
        phi = lambda t: jnp.where(t > 0, t + 1, jnp.exp(t)) + 1e-6
        pq, pk = phi(q), phi(k)
        kv = jnp.einsum("bhsd,bhse->bhde", pk, v)
        z = jnp.einsum("bhsd->bhd", pk)
        num = jnp.einsum("bhqd,bhde->bhqe", pq, kv)
        den = jnp.einsum("bhqd,bhd->bhq", pq, z)[..., None] + 1e-6
        o = num / den
        return (lambda x, *d: x.transpose(*d))(o, 0, 2, 1, 3).reshape(B, S, D) @ wo

    def _B_ref(x, w_r, w_gate, w_up, w_down):
        B, S, D = x.shape
        C = 1
        r = x @ w_r
        idx = jnp.argsort(-r, axis=-1)[:, :C]
        idx_e = jnp.repeat(idx.reshape(B, C, 1), D, axis=2)
        x_sel = jnp.take_along_axis(x, idx_e, axis=1)
        g = _silu(x_sel @ w_gate)
        u = x_sel @ w_up
        y = (g * u) @ w_down
        r_sel = _sigmoid(jnp.take_along_axis(r, idx, axis=1))
        y = y * r_sel.reshape(B, C, 1)
        b_off = (jnp.arange(B) * S).reshape(B, 1)
        flat_idx = (idx + b_off).reshape(B * C)
        zero = (x * 0.0).reshape(B * S, D)
        upd = _scatter_add(zero, flat_idx, y.reshape(B * C, D), axis=0)
        return x + upd.reshape(B, S, D)

    x = A_x
    g = _sigmoid((x * gate_w).sum(-1, keepdims=True))
    a = _A_ref(x, A_wqkv, A_wo)
    b = _B_ref(x, B_w_r, B_w_gate, B_w_up, B_w_down)
    return g * a + (1 - g) * b
```

```python
import jax
import jax.numpy as jnp
import jax.experimental.pallas as pl
import jax.experimental.pallas.tpu as pltpu

F32 = jnp.float32
BF16 = jnp.bfloat16

S = 2048
D = 1024
FF = 3584
DH = 32
TM = 512
NT = S // TM
DC = D // NT
FC = FF // NT
OM = 256
F32_MAX = 3.4028234663852886e38

NT_DIMS = (((1,), (1,)), ((), ()))
TN_DIMS = (((0,), (0,)), ((), ()))


def _phi(t):
    return jnp.where(t > 0, t + 1.0, jnp.exp(t)) + 1e-6


def _sigmoid(t):
    return 1.0 / (1.0 + jnp.exp(-t))


def _lanes(v, n):
    return v if n == 1 else jnp.concatenate([v] * n, axis=1)


def _fold_lanes(v):
    acc = v[:, 0:128]
    for j in range(1, v.shape[1] // 128):
        acc = acc + v[:, j * 128:(j + 1) * 128]
    return acc


def _as_column(row):
    tiles = [jnp.broadcast_to(row[:, j * 128:(j + 1) * 128], (128, 128)).T
             for j in range(row.shape[1] // 128)]
    return tiles[0] if len(tiles) == 1 else jnp.concatenate(tiles, axis=0)


def _matvec(w_ref, row0, col, acc, width):
    out = []
    for c, a in enumerate(acc):
        for g in range(col.shape[0] // 16):
            w = w_ref[row0 + 16 * g:row0 + 16 * g + 16, c * width:(c + 1) * width].astype(F32)
            p = w * _lanes(col[16 * g:16 * g + 16], width // 128)
            p = p[0:8] + p[8:16]
            a = p if a is None else a + p
        out.append(a)
    return out


def _row_vector(v_ref):
    v = v_ref[...].astype(F32)
    return jnp.concatenate([v[j:j + 1, :] for j in range(8)], axis=1)


def _kernel(x_hbm, wqkv_hbm, wo_hbm, wr_hbm, wg_hbm, wu_hbm, wd_hbm, gw_hbm, out_hbm,
            x_v, wk_v, wq_v, wv_v, wo_v, wg_v, wu_v, wd_v, wr_v, gw_v,
            wkt_v, wqt_v, p_v, g_v, m_v, out_v, sems):
    copies = {}

    def define(name, src, dst):
        copies[name] = pltpu.make_async_copy(src, dst, sems.at[len(copies)])

    for i in range(NT):
        rows = pl.ds(i * TM, TM)
        define(("x", i), x_hbm.at[rows, :], x_v.at[rows, :])
        define(("wq", i), wqkv_hbm.at[:, pl.ds(i * DC, DC)], wq_v.at[i])
        define(("wk", i), wqkv_hbm.at[:, pl.ds(D + i * DC, DC)], wk_v.at[i])
        define(("wg", i), wg_hbm.at[pl.ds(i * DC, DC), :], wg_v.at[pl.ds(i * DC, DC), :])
        define(("wu", i), wu_hbm.at[pl.ds(i * DC, DC), :], wu_v.at[pl.ds(i * DC, DC), :])
        define(("wd", i), wd_hbm.at[pl.ds(i * FC, FC), :], wd_v.at[pl.ds(i * FC, FC), :])
    for i in range(S // OM):
        rows = pl.ds(i * OM, OM)
        define(("out", i), out_v.at[rows, :], out_hbm.at[rows, :])
    define("wv", wqkv_hbm.at[:, pl.ds(2 * D, D)], wv_v)
    define("wo", wo_hbm, wo_v)
    define("wr", wr_hbm, wr_v)
    define("gw", gw_hbm, gw_v)

    def start(*names):
        for n in names:
            copies[n].start()

    def wait(*names):
        for n in names:
            copies[n].wait()

    start(("wk", 0), ("x", 0), ("wk", 1), ("wk", 2), ("wk", 3), "wr", "gw")

    def key_block(f0, nf, i):
        kt = jax.lax.dot_general(wkt_v[f0:f0 + nf, :], x_v[i * TM:(i + 1) * TM, :], NT_DIMS,
                                 preferred_element_type=F32)
        pk = _phi(kt)
        p_v[f0:f0 + nf, i * TM:(i + 1) * TM] = pk.astype(BF16)
        return _fold_lanes(pk)

    z_parts = []
    for c in range(NT):
        wait(("wk", c))
        wkt_v[c * DC:(c + 1) * DC, :] = wk_v[c].T
        if c == 0:
            wait(("x", 0))
        if c == NT - 1:
            start(("x", 1), ("x", 2), ("x", 3))
        z_parts.append(key_block(c * DC, DC, 0))
    z_acc = jnp.concatenate(z_parts, axis=0)

    wait("wr", "gw")
    wr_row = _row_vector(wr_v)
    sub = jax.lax.broadcasted_iota(jnp.int32, (8, 1), 0)
    best_key = jnp.full((8, 1), -jnp.inf, F32)
    best_idx = sub

    def route(r0, nr, best_key, best_idx):
        for g in range(nr // 64):
            t0 = r0 + g * 64
            r = jnp.sum(_fold_lanes(x_v[t0:t0 + 64, :].astype(F32) * wr_row), axis=1, keepdims=True)
            r = r.astype(BF16).astype(F32)
            key = jnp.where(r != r, -jnp.inf, jnp.maximum(r, -F32_MAX))
            for k in range(8):
                kk = key[8 * k:8 * k + 8]
                better = kk > best_key
                best_key = jnp.where(better, kk, best_key)
                best_idx = jnp.where(better, sub + (t0 + 8 * k), best_idx)
        return best_key, best_idx

    for i in range(1, NT):
        if i == 1:
            wait(("x", 1))
        elif i == 2:
            wait(("x", 2), ("x", 3))
        start(("wg", i - 1), ("wu", i - 1), ("wq", i - 1))
        z_acc = z_acc + key_block(0, D, i)
        if i < 3:
            best_key, best_idx = route((i - 1) * (S // 2), S // 2, best_key, best_idx)
        else:
            top = jnp.max(best_key, axis=0, keepdims=True)
            idx = jnp.min(jnp.where(best_key == top, best_idx, S))
            grp = x_v[pl.ds(pl.multiple_of((idx // 16) * 16, 16), 16), :].astype(F32)
            hit = jax.lax.broadcasted_iota(jnp.int32, (16, D), 0) == idx % 16
            x_sel = jnp.sum(jnp.where(hit, grp, 0.0), axis=0, keepdims=True)
            r_sel = jnp.sum(x_sel * wr_row, axis=1, keepdims=True)
    z_col = jnp.broadcast_to(jnp.sum(z_acc, axis=1, keepdims=True), (D, 128))

    acc_g = [None] * 4
    acc_u = [None] * 4
    for i in range(NT):
        wait(("wg", i), ("wu", i), ("wq", i))
        if i == 0:
            start(("wg", 3), ("wu", 3), ("wq", 3))
        elif i == 1:
            start("wv", "wo")
        elif i == 2:
            start(("wd", 0), ("wd", 1))
        else:
            start(("wd", 2), ("wd", 3))
        f0 = i * DC
        g_v[f0:f0 + DC, :] = jnp.dot(p_v[f0:f0 + DC, :], x_v[...],
                                     preferred_element_type=F32).astype(BF16)
        wqt_v[f0:f0 + DC, :] = wq_v[i].T
        col = _as_column(x_sel[:, f0:f0 + DC])
        acc_g = _matvec(wg_v, f0, col, acc_g, FF // 4)
        acc_u = _matvec(wu_v, f0, col, acc_u, FF // 4)
    gate = jnp.sum(jnp.concatenate(acc_g, axis=1), axis=0, keepdims=True)
    up = jnp.sum(jnp.concatenate(acc_u, axis=1), axis=0, keepdims=True)
    hidden = gate * _sigmoid(gate) * up

    same_head = (jax.lax.broadcasted_iota(jnp.int32, (128, 128), 0) // DH
                 == jax.lax.broadcasted_iota(jnp.int32, (128, 128), 1) // DH)
    acc_y = [None]
    wait("wv", "wo")
    for i in range(NT):
        wait(("wd", i))
        for j in range(i * DC // 128, (i + 1) * DC // 128):
            blk = slice(j * 128, (j + 1) * 128)
            kv = jnp.dot(g_v[blk, :], wv_v[:, blk], preferred_element_type=F32)
            kv = jnp.where(same_head, kv, 0.0).astype(BF16)
            m_v[blk, :] = jnp.dot(kv, wo_v[blk, :], preferred_element_type=F32).astype(BF16)
        qt = jax.lax.dot_general(wqt_v[...], x_v[i * TM:(i + 1) * TM, :], NT_DIMS,
                                 preferred_element_type=F32)
        pq = _phi(qt)
        den = jnp.sum((pq * _lanes(z_col, TM // 128)).reshape(D // DH, DH, TM),
                      axis=1, keepdims=True) + 1e-6
        pn = pq.reshape(D // DH, DH, TM) * (1.0 / den)
        p_v[:, i * TM:(i + 1) * TM] = pn.reshape(D, TM).astype(BF16)
        acc_y = _matvec(wd_v, i * FC, _as_column(hidden[:, i * FC:(i + 1) * FC]), acc_y, D)
    y = jnp.sum(acc_y[0], axis=0, keepdims=True) * _sigmoid(r_sel)

    gw_row = _row_vector(gw_v)
    for i in range(S // OM):
        rows = slice(i * OM, (i + 1) * OM)
        a = jax.lax.dot_general(p_v[:, rows], m_v[...], TN_DIMS, preferred_element_type=F32)
        xb = x_v[rows, :].astype(F32)
        g = _sigmoid(jnp.sum(_fold_lanes(xb * gw_row), axis=1, keepdims=True))
        tok = jax.lax.broadcasted_iota(jnp.int32, (OM, D), 0) + i * OM
        b = xb + (xb * 0.0 + jnp.where(tok == idx, y, 0.0))
        out_v[rows, :] = (g * a + (1.0 - g) * b).astype(BF16)
        start(("out", i))
    wait(*[("out", i) for i in range(S // OM)])


_NUM_COPIES = 6 * NT + S // OM + 4


@jax.jit
def pallas_gated_mix__linear_attn_block__moe_arch_mod__prompt_kernel(
    A_x: jax.Array,
    A_wqkv: jax.Array,
    A_wo: jax.Array,
    B_x: jax.Array,
    B_w_r: jax.Array,
    B_w_gate: jax.Array,
    B_w_up: jax.Array,
    B_w_down: jax.Array,
    gate_w: jax.Array,
):
    assert A_x.shape == (1, S, D) and B_w_gate.shape == (D, FF)
    hbm = pl.BlockSpec(memory_space=pl.ANY)
    out = pl.pallas_call(
        _kernel,
        out_shape=jax.ShapeDtypeStruct((S, D), BF16),
        in_specs=[hbm] * 8,
        out_specs=hbm,
        scratch_shapes=[
            pltpu.VMEM((S, D), BF16),
            pltpu.VMEM((NT, D, DC), BF16),
            pltpu.VMEM((NT, D, DC), BF16),
            pltpu.VMEM((D, D), BF16),
            pltpu.VMEM((D, D), BF16),
            pltpu.VMEM((D, FF), BF16),
            pltpu.VMEM((D, FF), BF16),
            pltpu.VMEM((FF, D), BF16),
            pltpu.VMEM((8, 128), BF16),
            pltpu.VMEM((8, 128), BF16),
            pltpu.VMEM((D, D), BF16),
            pltpu.VMEM((D, D), BF16),
            pltpu.VMEM((D, S), BF16),
            pltpu.VMEM((D, D), BF16),
            pltpu.VMEM((D, D), BF16),
            pltpu.VMEM((S, D), BF16),
            pltpu.SemaphoreType.DMA((_NUM_COPIES,)),
        ],
        compiler_params=pltpu.CompilerParams(vmem_limit_bytes=110 * 1024 * 1024),
        name="gated_mix_linear_attn_mod",
    )(A_x.reshape(S, D), A_wqkv, A_wo, B_w_r.reshape(8, 128),
      B_w_gate, B_w_up, B_w_down, gate_w.reshape(8, 128))
    return out.reshape(1, S, D)
```

```python
import os
import jax
import jax.numpy as jnp
import jax.experimental.pallas as pl
import jax.experimental.pallas.tpu as pltpu

F32 = jnp.float32
BF16 = jnp.bfloat16

def eval_pair(k, d):
    return tuple(int(v) for v in os.environ.get(k, d).split(','))


SIDE = int(os.environ.get('SIDE', 1))
SCOPES = int(os.environ.get('SCOPES', 0))
MR, DR = eval_pair('MDR', '32,32')
QM, QN = eval_pair('QMN', '256,512')
LAG = int(os.environ.get('LAG', 1))
PRO = int(os.environ.get('PRO', 1))
X_PARTS = ((0, 256), (256, 512), (512, 1024), (1024, 2048)) if PRO else ((0, 512), (512, 2048))
OUT_PARTS = tuple((k, 0, 256) for k in range(7)) + ((7, 0, 128), (7, 128, 128))
WK_PARTS = ((0, 256), (256, 512), (512, 1024)) if PRO else ((0, 256), (256, 1024))
MEND = int(os.environ.get('MEND', 1))
S = 2048
D = 1024
FF = 3584
DH = 32
TM = 512
NT = S // TM
DC = D // NT
FC = int(os.environ.get('FC', 512))
FU = int(os.environ.get('FU', 1536))
OM = 256
PM, PN = eval_pair('PMN', '256,512')
GM, GN = eval_pair('GMN', '256,1024')
F32_MAX = 3.4028234663852886e38

NT_DIMS = (((1,), (1,)), ((), ()))
TN_DIMS = (((0,), (0,)), ((), ()))


def _phi(t):
    return jnp.where(t > 0, t + 1.0, jnp.exp(t)) + 1e-6


def _sigmoid(t):
    return 1.0 / (1.0 + jnp.exp(-t))


def _lanes(v, n):
    return v if n == 1 else jnp.concatenate([v] * n, axis=1)


def _fold_lanes(v):
    acc = v[:, 0:128]
    for j in range(1, v.shape[1] // 128):
        acc = acc + v[:, j * 128:(j + 1) * 128]
    return acc


def _as_column(row):
    tiles = [jnp.broadcast_to(row[:, j * 128:(j + 1) * 128], (128, 128)).T
             for j in range(row.shape[1] // 128)]
    return tiles[0] if len(tiles) == 1 else jnp.concatenate(tiles, axis=0)


def _interleave(main, side=(), carry=None):
    pending, done, due = carry, 0, {}
    for k, piece in enumerate(main):
        epilogue = piece()
        if pending is not None:
            pending()
        pending = epilogue
        upto = (k + 1) * len(side) // len(main)
        due[k + LAG] = [job() for job in side[done:upto]]
        done = upto
        for deadline in due.pop(k, ()):
            if callable(deadline):
                deadline()
    return pending


def _row_vector(v_ref):
    v = v_ref[...].astype(F32)
    return jnp.concatenate([v[j:j + 1, :] for j in range(8)], axis=1)


def _kernel(x_hbm, wqkv_hbm, wo_hbm, wr_hbm, wg_hbm, wu_hbm, wd_hbm, gw_hbm, out_hbm,
            x_v, wk_v, wq_v, wv_v, wo_v, wg_v, wu_v, wd_v, wr_v, gw_v,
            wkt_v, p_v, q_v, g_v, m_v, xcol_v, hcol_v, sems):
    copies = {}

    def define(name, src, dst):
        copies[name] = pltpu.make_async_copy(src, dst, sems.at[len(copies)])

    for i, (t0, t1) in enumerate(X_PARTS):
        define(("x", i), x_hbm.at[pl.ds(t0, t1 - t0), :], x_v.at[pl.ds(t0, t1 - t0), :])
    for i, (c0, c1) in enumerate(WK_PARTS):
        define(("wk", i), wqkv_hbm.at[:, pl.ds(D + c0, c1 - c0)], wk_v.at[:, pl.ds(c0, c1 - c0)])
    for i, cols in enumerate((pl.ds(0, FU), pl.ds(FU, FF - FU))):
        define(("wu", i), wu_hbm.at[:, cols], wu_v.at[pl.ds(0, D), cols])
    define("wg", wg_hbm, wg_v.at[pl.ds(0, D), :])
    define("wd", wd_hbm, wd_v.at[pl.ds(0, FF), :])
    define("wq", wqkv_hbm.at[:, pl.ds(0, D)], wq_v)
    define("wv", wqkv_hbm.at[:, pl.ds(2 * D, D)], wv_v)
    define("wo", wo_hbm, wo_v)
    define("wr", wr_hbm, wr_v)
    define("gw", gw_hbm, gw_v)

    def start(*names):
        for n in names:
            copies[n].start()

    scope = []

    def wait(*names):
        if SCOPES:
            if scope:
                scope.pop().__exit__(None, None, None)
            with jax.named_scope("wait_" + str(names[0]).replace(" ", "")):
                for n in names:
                    copies[n].wait()
            scope.append(jax.named_scope("after_" + str(names[0]).replace(" ", "")))
            scope[-1].__enter__()
            return
        for n in names:
            copies[n].wait()

    z_acc = {}

    def key_piece(f0, t0, PM=PM, PN=PN):
        def piece():
            kt = jax.lax.dot_general(wkt_v[f0:f0 + PM, :], x_v[t0:t0 + PN, :], NT_DIMS,
                                     preferred_element_type=F32)

            def epilogue():
                pk = _phi(kt)
                p_v[f0:f0 + PM, t0:t0 + PN] = pk.astype(BF16)
                part = _fold_lanes(pk)
                for f in range(0, PM, 128):
                    old = z_acc.get(f0 + f)
                    z_acc[f0 + f] = part[f:f + 128] if old is None else old + part[f:f + 128]
            return epilogue
        return piece

    def transpose_wk(c):
        wkt_v[c * DC:(c + 1) * DC, :] = wk_v[:, c * DC:(c + 1) * DC].T

    later = ("wr", "gw", "wg", ("wu", 0), ("wu", 1), "wq", "wv", "wo", "wd")
    if PRO:
        start(("wk", 0), ("x", 0), ("wk", 1), ("x", 1), ("wk", 2), ("x", 2), ("x", 3), *later)
        wait(("wk", 0))
        transpose_wk(0)
        wait(("x", 0))
        last = _interleave([key_piece(0, 0, DC, 256)])
        wait(("wk", 1), ("x", 1))
        transpose_wk(1)
        last = _interleave([key_piece(0, 256, DC, 256), key_piece(DC, 0, DC, TM)], carry=last)
        wait(("wk", 2))
        transpose_wk(2)
        transpose_wk(3)
        last = _interleave([key_piece(c * DC, 0, DC, TM) for c in (2, 3)], carry=last)
    else:
        start(("wk", 0), ("x", 0), ("wk", 1), ("x", 1), *later)
        wait(("wk", 0))
        transpose_wk(0)
        wait(("x", 0))
        last = _interleave([key_piece(0, 0, DC, TM)])
        wait(("wk", 1))
        for c in range(1, NT):
            transpose_wk(c)
            last = _interleave([key_piece(c * DC, 0, DC, TM)], carry=last)

    if PRO:
        wait(("x", 2))
        last = _interleave([key_piece(f0, TM) for f0 in range(0, D, PM)], carry=last)
    wait(("x", len(X_PARTS) - 1), "wr")
    wr_row = _row_vector(wr_v)
    sub = jax.lax.broadcasted_iota(jnp.int32, (8, 1), 0)
    route = {"key": jnp.full((8, 1), -jnp.inf, F32), "idx": sub}

    def route_job(t0):
        def job():
            r = jnp.sum(_fold_lanes(x_v[t0:t0 + 64, :].astype(F32) * wr_row), axis=1, keepdims=True)
            r = r.astype(BF16).astype(F32)
            key = jnp.where(r != r, -jnp.inf, jnp.maximum(r, -F32_MAX))
            for k in range(8):
                kk = key[8 * k:8 * k + 8]
                better = kk > route["key"]
                route["key"] = jnp.where(better, kk, route["key"])
                route["idx"] = jnp.where(better, sub + (t0 + 8 * k), route["idx"])
        return job

    def select_job():
        top = jnp.max(route["key"], axis=0, keepdims=True)
        idx = jnp.min(jnp.where(route["key"] == top, route["idx"], S))
        grp = x_v[pl.ds(pl.multiple_of((idx // 16) * 16, 16), 16), :].astype(F32)
        hit = jax.lax.broadcasted_iota(jnp.int32, (16, D), 0) == idx % 16
        route["token"] = idx
        route["x"] = jnp.sum(jnp.where(hit, grp, 0.0), axis=0, keepdims=True)
        route["score"] = jnp.sum(route["x"] * wr_row, axis=1, keepdims=True)

    idle = [lambda: None]
    last = _interleave([key_piece(f0, t0) for t0 in range(2 * TM if PRO else TM, S, PN) for f0 in range(0, D, PM)],
               [route_job(t0) for t0 in range(0, S if SIDE else 64, 64)] + [select_job] + idle * 8, carry=last)

    acc = {}
    zero = pl.multiple_of((route["token"] // S) * 16, 16)

    def pace(w_ref, value):
        w_ref[w_ref.shape[0] - 16:, 0:128] = value[0:16, 0:128].astype(BF16)

    def column_job(col_ref, row, j):
        def job():
            col_ref[j * 128:(j + 1) * 128, :] = _as_column(row[:, j * 128:(j + 1) * 128])
        return job

    def matvec_job(name, w_ref, col_ref, r0, nr, c0, width, lhs_ref):
        def job():
            a = acc.get((name, c0))
            for r in range(r0, r0 + nr, 16):
                w = w_ref[pl.ds(zero + r, 16), c0:c0 + width].astype(F32)
                p = w * _lanes(col_ref[r:r + 16, :], width // 128)
                p = p[0:8] + p[8:16]
                a = p if a is None else a + p
            acc[name, c0] = a
            for ref in lhs_ref:
                pace(ref, jnp.concatenate([_fold_lanes(a)] * 2, axis=0))
        return job

    def g_piece(f0, d0):
        def piece():
            g = jnp.dot(p_v[f0:f0 + GM, :], x_v[:, d0:d0 + GN], preferred_element_type=F32)

            def epilogue():
                g_v[f0:f0 + GM, d0:d0 + GN] = g.astype(BF16)
            return epilogue
        return piece

    for j in range(D // 128):
        column_job(xcol_v, route["x"], j)()
    wait("wg", ("wu", 0))

    def ffn_in_jobs(name, w_ref, c0):
        return [matvec_job(name, w_ref, xcol_v, r0, MR, c0, FC, (w_ref,)) for r0 in range(0, D, MR)]

    side = []
    for c0 in range(0, FF, FC):
        side += ffn_in_jobs("gate", wg_v, c0)
    for c0 in range(0, FU, FC):
        side += ffn_in_jobs("up", wu_v, c0)
    last = _interleave([g_piece(f0, d0) for f0 in range(0, D, GM) for d0 in range(0, D, GN)],
                       side, carry=last)

    def total(name, c0):
        return jnp.sum(acc[name, c0], axis=0, keepdims=True)

    def hidden_job(c0):
        def job():
            gate = total("gate", c0)
            hcol_v[c0:c0 + FC, :] = _as_column(gate * _sigmoid(gate) * total("up", c0))
        return job

    z_col = {f0: jnp.broadcast_to(jnp.sum(z, axis=1, keepdims=True), (128, 128))
             for f0, z in z_acc.items()}

    same_head = (jax.lax.broadcasted_iota(jnp.int32, (128, 128), 0) // DH
                 == jax.lax.broadcasted_iota(jnp.int32, (128, 128), 1) // DH)

    def query_piece(f0, t0, PM=DC, PN=QN):
        def piece():
            qt = jax.lax.dot_general(wq_v[:, f0:f0 + PM], x_v[t0:t0 + PN, :], (((0,), (1,)), ((), ())),
                                     preferred_element_type=F32)

            def epilogue():
                pq = _phi(qt)
                den = jnp.sum((pq * _lanes(jnp.concatenate([z_col[f0 + f] for f in range(0, PM, 128)], axis=0), PN // 128)).reshape(PM // DH, DH, PN),
                              axis=1, keepdims=True) + 1e-6
                pn = pq.reshape(PM // DH, DH, PN) * (1.0 / den)
                q_v[t0:t0 + PN, f0:f0 + PM] = pn.reshape(PM, PN).astype(BF16).T
            return epilogue
        return piece

    kv = {}

    def kv_job(j):
        def job():
            blk = slice(j * 128, (j + 1) * 128)
            full = jnp.dot(g_v[blk, :], wv_v[:, blk], preferred_element_type=F32)
            kv[j] = jnp.where(same_head, full, 0.0).astype(BF16)
        return job

    def m_job(j):
        def job():
            blk = slice(j * 128, (j + 1) * 128)
            m_v[blk, :] = jnp.dot(kv[j], wo_v[blk, :], preferred_element_type=F32).astype(BF16)
        return job

    last()
    wait(("wu", 1), "wq", "wv", "wo")
    side = []
    for c0 in range(FU, FF, FC):
        side += ffn_in_jobs("up", wu_v, c0)
    side += [hidden_job(c0) for c0 in range(0, FF, FC)]
    main = [query_piece(f0, t0) for f0 in range(0, D, DC) for t0 in range(0, S, QN)]
    small = [kv_job(0)] + [job for j in range(1, 8) for job in (kv_job(j), m_job(j - 1))] + [m_job(7)]
    if MEND:
        main += small
    else:
        step = len(side) // 16
        for j in reversed(range(16)):
            side.insert(j * step, small[j])
    last = _interleave(main, side)
    if last is not None:
        last()

    wait("wd", "gw")
    gw_row = _row_vector(gw_v)
    last_tile = route["token"] // OM

    def out_piece(i):
        def piece():
            k, r0, nr = OUT_PARTS[i]
            t0 = pl.multiple_of(((last_tile + 1 + k) % (S // OM)) * OM + r0, 128)
            rows = pl.ds(t0, nr)
            a = jnp.dot(q_v[rows, :], m_v[...], preferred_element_type=F32)

            def epilogue():
                xb = x_v[rows, :].astype(F32)
                g = _sigmoid(jnp.sum(_fold_lanes(xb * gw_row), axis=1, keepdims=True))
                upd = xb * 0.0
                if k == S // OM - 1:
                    y = jnp.concatenate([total("down", n0) for n0 in range(0, D, FC)], axis=1)
                    tok = jax.lax.broadcasted_iota(jnp.int32, (nr, D), 0) + t0
                    upd = upd + jnp.where(tok == route["token"], y * _sigmoid(route["score"]), 0.0)
                x_v[rows, :] = (g * a + (1.0 - g) * (xb + upd)).astype(BF16)
                define(("out", i), x_v.at[rows, :], out_hbm.at[rows, :])
                start(("out", i))
            return epilogue
        return piece

    side = [matvec_job("down", wd_v, hcol_v, r0, DR, n0, FC, (wd_v,))
            for n0 in range(0, D, FC) for r0 in range(0, FF, DR)]
    last = _interleave([out_piece(i) for i in range(len(OUT_PARTS) - 2)], side)
    last = _interleave([out_piece(i) for i in range(len(OUT_PARTS) - 2, len(OUT_PARTS))], carry=last)
    last()
    wait(*[("out", i) for i in range(len(OUT_PARTS))])
    if scope:
        scope.pop().__exit__(None, None, None)


_NUM_COPIES = len(WK_PARTS) + len(X_PARTS) + len(OUT_PARTS) + 9


@jax.jit
def pallas_gated_mix__linear_attn_block__moe_arch_mod__prompt_kernel(
    A_x: jax.Array,
    A_wqkv: jax.Array,
    A_wo: jax.Array,
    B_x: jax.Array,
    B_w_r: jax.Array,
    B_w_gate: jax.Array,
    B_w_up: jax.Array,
    B_w_down: jax.Array,
    gate_w: jax.Array,
):
    assert A_x.shape == (1, S, D) and B_w_gate.shape == (D, FF)
    hbm = pl.BlockSpec(memory_space=pl.ANY)
    out = pl.pallas_call(
        _kernel,
        out_shape=jax.ShapeDtypeStruct((S, D), BF16),
        in_specs=[hbm] * 8,
        out_specs=hbm,
        scratch_shapes=[
            pltpu.VMEM((S, D), BF16),
            pltpu.VMEM((D, D), BF16),
            pltpu.VMEM((D, D), BF16),
            pltpu.VMEM((D, D), BF16),
            pltpu.VMEM((D, D), BF16),
            pltpu.VMEM((D + 16, FF), BF16),
            pltpu.VMEM((D + 16, FF), BF16),
            pltpu.VMEM((FF + 16, D), BF16),
            pltpu.VMEM((8, 128), BF16),
            pltpu.VMEM((8, 128), BF16),
            pltpu.VMEM((D, D), BF16),
            pltpu.VMEM((D, S), BF16),
            pltpu.VMEM((S, D), BF16),
            pltpu.VMEM((D, D), BF16),
            pltpu.VMEM((D, D), BF16),
            pltpu.VMEM((D, 128), F32),
            pltpu.VMEM((FF, 128), F32),
            pltpu.SemaphoreType.DMA((_NUM_COPIES,)),
        ],
        compiler_params=pltpu.CompilerParams(vmem_limit_bytes=110 * 1024 * 1024,
            flags={k: True for k in os.environ.get('FL', 'XLA_TPU_EVENLY_DISTRIBUTE_CRITICAL_NODES').split(',') if k}),
        name="gated_mix_linear_attn_mod",
    )(A_x.reshape(S, D), A_wqkv, A_wo, B_w_r.reshape(8, 128),
      B_w_gate, B_w_up, B_w_down, gate_w.reshape(8, 128))
    return out.reshape(1, S, D)
```

```python
import jax
import jax.numpy as jnp
import jax.experimental.pallas as pl
import jax.experimental.pallas.tpu as pltpu

F32 = jnp.float32
BF16 = jnp.bfloat16

S = 2048
D = 1024
FF = 3584
DH = 32
PF = 256
PT = 512
GF = 512
MR = 32
MC = 512
X_PARTS = ((0, 256), (256, 512), (512, 1024), (1024, 2048))
WK_PARTS = ((0, 256), (256, 512), (512, 1024))
OUT_PARTS = ((0, 0, 512), (1, 0, 512), (2, 0, 512), (3, 0, 320), (3, 320, 128), (3, 448, 64))
NUM_COPIES = len(X_PARTS) + len(WK_PARTS) + len(OUT_PARTS) + 8
F32_MAX = 3.4028234663852886e38

NT_DIMS = (((1,), (1,)), ((), ()))
TT_DIMS = (((0,), (1,)), ((), ()))


def _phi(t):
    return jnp.where(t > 0, t + 1.0, jnp.exp(t)) + 1e-6


def _sigmoid(t):
    return 1.0 / (1.0 + jnp.exp(-t))


def _lanes(v, n):
    return v if n == 1 else jnp.concatenate([v] * n, axis=1)


def _fold_lanes(v):
    acc = v[:, 0:128]
    for j in range(1, v.shape[1] // 128):
        acc = acc + v[:, j * 128:(j + 1) * 128]
    return acc


def _as_column(row):
    tiles = [jnp.broadcast_to(row[:, j * 128:(j + 1) * 128], (128, 128)).T
             for j in range(row.shape[1] // 128)]
    return tiles[0] if len(tiles) == 1 else jnp.concatenate(tiles, axis=0)


def _row_vector(v_ref):
    v = v_ref[...].astype(F32)
    return jnp.concatenate([v[j:j + 1, :] for j in range(8)], axis=1)


def _interleave(main, side=(), carry=None):
    pending, done = carry, 0
    for k, piece in enumerate(main):
        epilogue = piece()
        if pending is not None:
            pending()
        pending = epilogue
        upto = (k + 1) * len(side) // len(main)
        for job in side[done:upto]:
            job()
        done = upto
    return pending


def _kernel(x_hbm, wqkv_hbm, wo_hbm, wr_hbm, wg_hbm, wu_hbm, wd_hbm, gw_hbm, out_hbm,
            x_v, wk_v, wq_v, wv_v, wo_v, wg_v, wu_v, wd_v, wr_v, gw_v,
            wkt_v, wqt_v, pk_v, pq_v, g_v, m_v, xcol_v, hcol_v, mix_v, sems):
    copies = {}

    def define(name, src, dst):
        copies[name] = pltpu.make_async_copy(src, dst, sems.at[len(copies)])

    def start(*names):
        for n in names:
            copies[n].start()

    def wait(*names):
        for n in names:
            copies[n].wait()

    for i, (t0, t1) in enumerate(X_PARTS):
        define(("x", i), x_hbm.at[pl.ds(t0, t1 - t0), :], x_v.at[pl.ds(t0, t1 - t0), :])
    for i, (c0, c1) in enumerate(WK_PARTS):
        define(("wk", i), wqkv_hbm.at[:, pl.ds(D + c0, c1 - c0)], wk_v.at[:, pl.ds(c0, c1 - c0)])
    define("wq", wqkv_hbm.at[:, pl.ds(0, D)], wq_v)
    define("wv", wqkv_hbm.at[:, pl.ds(2 * D, D)], wv_v)
    define("wo", wo_hbm, wo_v)
    define("wg", wg_hbm, wg_v.at[pl.ds(0, D), :])
    define("wu", wu_hbm, wu_v.at[pl.ds(0, D), :])
    define("wd", wd_hbm, wd_v.at[pl.ds(0, FF), :])
    define("wr", wr_hbm, wr_v)
    define("gw", gw_hbm, gw_v)

    z_acc = {}

    def key_piece(f0, t0, nt=PT, transposed=True):
        def piece():
            if transposed:
                kt = jax.lax.dot_general(wkt_v[f0:f0 + PF, :], x_v[t0:t0 + nt, :], NT_DIMS,
                                         preferred_element_type=F32)
            else:
                kt = jax.lax.dot_general(wk_v[:, f0:f0 + PF], x_v[t0:t0 + nt, :], TT_DIMS,
                                         preferred_element_type=F32)

            def epilogue():
                pk = _phi(kt)
                pk_v[f0:f0 + PF, t0:t0 + nt] = pk.astype(BF16)
                part = _fold_lanes(pk)
                z_acc[f0] = z_acc[f0] + part if f0 in z_acc else part
            return epilogue
        return piece

    def transpose_job(src_v, dst_v, f0):
        def job():
            dst_v[f0:f0 + PF, :] = src_v[:, f0:f0 + PF].T
        return job

    start(("wk", 0), ("x", 0), ("x", 1), ("wk", 1), ("wk", 2), ("x", 2), ("x", 3),
          "wr", "gw", "wg", "wq", "wv", "wo", "wu", "wd")
    wait(("wk", 0), ("x", 0))
    last = _interleave([key_piece(0, 0, 256, False)])
    wait(("x", 1))
    last = _interleave([key_piece(0, 256, 256, False)], carry=last)
    wait(("wk", 1))
    last = _interleave([key_piece(PF, 0, PT, False)], carry=last)
    wait(("wk", 2))
    last = _interleave([key_piece(f0, 0, PT, False) for f0 in (2 * PF, 3 * PF)],
                       [transpose_job(wk_v, wkt_v, f0) for f0 in range(0, D, PF)], carry=last)
    wait(("x", 2))
    last = _interleave([key_piece(f0, PT) for f0 in range(0, D, PF)], carry=last)
    wait(("x", 3), "wr", "gw")

    wr_row = _row_vector(wr_v)
    gw_row = _row_vector(gw_v)
    sub = jax.lax.broadcasted_iota(jnp.int32, (8, 1), 0)
    best = [jnp.full((8, 1), -jnp.inf, F32), sub]

    def score_job(t0):
        def job():
            xf = x_v[t0:t0 + 64, :].astype(F32)
            g = _sigmoid(jnp.sum(_fold_lanes(xf * gw_row), axis=1, keepdims=True))
            mix_v[t0:t0 + 64, :] = jnp.broadcast_to(g, (64, 128))
            r = jnp.sum(_fold_lanes(xf * wr_row), axis=1, keepdims=True)
            r = r.astype(BF16).astype(F32)
            key = jnp.where(r != r, -jnp.inf, jnp.maximum(r, -F32_MAX))
            for k in range(0, 64, 8):
                better = key[k:k + 8] > best[0]
                best[0] = jnp.where(better, key[k:k + 8], best[0])
                best[1] = jnp.where(better, sub + (t0 + k), best[1])
        return job

    routed = {}

    def select_job():
        top = jnp.max(best[0], axis=0, keepdims=True)
        token = jnp.min(jnp.where(best[0] == top, best[1], S))
        group = x_v[pl.ds(pl.multiple_of((token // 16) * 16, 16), 16), :].astype(F32)
        hit = jax.lax.broadcasted_iota(jnp.int32, (16, D), 0) == token % 16
        routed["token"] = token
        routed["x"] = jnp.sum(jnp.where(hit, group, 0.0), axis=0, keepdims=True)

    last = _interleave([key_piece(f0, t0) for t0 in range(2 * PT, S, PT) for f0 in range(0, D, PF)],
                       [score_job(t0) for t0 in range(0, S, 64)] + [select_job] + [lambda: None] * 8,
                       carry=last)
    token, x_sel = routed["token"], routed["x"]
    weight = _sigmoid(jnp.sum(x_sel * wr_row, axis=1, keepdims=True))

    zero = pl.multiple_of((token // S) * 16, 16)
    acc = {}

    def matvec_job(name, w_v, col_v, r0, c0):
        def job():
            a = acc.get((name, c0))
            for r in range(r0, r0 + MR, 8):
                w = w_v[pl.ds(zero + r, 8), c0:c0 + MC].astype(F32)
                p = w * _lanes(col_v[r:r + 8, :], MC // 128)
                a = p if a is None else a + p
            acc[name, c0] = a
            w_v[w_v.shape[0] - 16:, 0:128] = jnp.concatenate([_fold_lanes(a)] * 2, axis=0).astype(BF16)
        return job

    def matvec_jobs(name, w_v, col_v):
        return [matvec_job(name, w_v, col_v, r0, c0)
                for c0 in range(0, w_v.shape[1], MC) for r0 in range(0, col_v.shape[0], MR)]

    def total(name, c0):
        return jnp.sum(acc[name, c0], axis=0, keepdims=True)

    def token_column_job(c0):
        def job():
            xcol_v[c0:c0 + 128, :] = _as_column(x_sel[:, c0:c0 + 128])
        return job

    def hidden_job(c0):
        def job():
            gate = total("gate", c0)
            hcol_v[c0:c0 + MC, :] = _as_column(gate * _sigmoid(gate) * total("up", c0))
        return job

    def g_piece(f0):
        def piece():
            g = jnp.dot(pk_v[f0:f0 + GF, :], x_v[...], preferred_element_type=F32)

            def epilogue():
                g_v[f0:f0 + GF, :] = g.astype(BF16)
            return epilogue
        return piece

    last = _interleave([g_piece(0)], [token_column_job(c0) for c0 in range(0, D, 128)], carry=last)
    wait("wg", "wq", "wv", "wo")
    last = _interleave([g_piece(f0) for f0 in range(GF, D, GF)],
                       matvec_jobs("gate", wg_v, xcol_v)
                       + [transpose_job(wq_v, wqt_v, f0) for f0 in range(0, D, PF)], carry=last)
    z_col = {f0: jnp.broadcast_to(jnp.sum(z, axis=1, keepdims=True), (PF, 128))
             for f0, z in z_acc.items()}

    def query_piece(f0, t0):
        def piece():
            qt = jax.lax.dot_general(wqt_v[f0:f0 + PF, :], x_v[t0:t0 + PT, :], NT_DIMS,
                                     preferred_element_type=F32)

            def epilogue():
                pq = _phi(qt)
                den = jnp.sum((pq * _lanes(z_col[f0], PT // 128)).reshape(PF // DH, DH, PT),
                              axis=1, keepdims=True) + 1e-6
                pn = pq.reshape(PF // DH, DH, PT) * (1.0 / den)
                pq_v[t0:t0 + PT, f0:f0 + PF] = pn.reshape(PF, PT).astype(BF16).T
            return epilogue
        return piece

    same_head = (jax.lax.broadcasted_iota(jnp.int32, (128, 128), 0) // DH
                 == jax.lax.broadcasted_iota(jnp.int32, (128, 128), 1) // DH)
    kv = {}

    def kv_job(f0):
        def job():
            full = jnp.dot(g_v[f0:f0 + 128, :], wv_v[:, f0:f0 + 128], preferred_element_type=F32)
            kv[f0] = jnp.where(same_head, full, 0.0).astype(BF16)
        return job

    def m_job(f0):
        def job():
            m_v[f0:f0 + 128, :] = jnp.dot(kv[f0], wo_v[f0:f0 + 128, :],
                                          preferred_element_type=F32).astype(BF16)
        return job

    late = 5 * 128
    last = _interleave([query_piece(f0, t0) for t0 in range(0, S, PT) for f0 in range(0, D, PF)],
                       [job for f0 in range(0, D, 128)
                        for job in [kv_job(f0)] + ([m_job(f0)] if f0 < late else [])], carry=last)
    last = _interleave([m_job(f0) for f0 in range(late, D, 128)], carry=last)
    assert last is None

    wait("wu", "wd")
    tiles = S // PT

    def out_piece(i):
        def piece():
            k, r0, nr = OUT_PARTS[i]
            t0 = pl.multiple_of(((token // PT + 1 + k) % tiles) * PT + r0, 64)
            rows = pl.ds(t0, nr)
            a = jnp.dot(pq_v[rows, :], m_v[...], preferred_element_type=F32)

            def epilogue():
                xf = x_v[rows, :].astype(F32)
                g = mix_v[rows, :]
                upd = xf * 0.0
                if k == tiles - 1:
                    y = jnp.concatenate([total("down", c0) for c0 in range(0, D, MC)], axis=1) * weight
                    is_token = jax.lax.broadcasted_iota(jnp.int32, (nr, D), 0) + t0 == token
                    upd = upd + jnp.where(is_token, y, 0.0)
                mixed = _lanes(g, D // 128) * a + _lanes(1.0 - g, D // 128) * (xf + upd)
                x_v[rows, :] = mixed.astype(BF16)
                define(("out", i), x_v.at[rows, :], out_hbm.at[rows, :])
                start(("out", i))
            return epilogue
        return piece

    last = _interleave([out_piece(i) for i in range(len(OUT_PARTS) - 2)],
                       matvec_jobs("up", wu_v, xcol_v) + [hidden_job(c0) for c0 in range(0, FF, MC)]
                       + matvec_jobs("down", wd_v, hcol_v))
    last = _interleave([out_piece(i) for i in range(len(OUT_PARTS) - 2, len(OUT_PARTS))], carry=last)
    last()
    wait(*[("out", i) for i in range(len(OUT_PARTS))])


@jax.jit
def pallas_gated_mix__linear_attn_block__moe_arch_mod__prompt_kernel(
    A_x: jax.Array,
    A_wqkv: jax.Array,
    A_wo: jax.Array,
    B_x: jax.Array,
    B_w_r: jax.Array,
    B_w_gate: jax.Array,
    B_w_up: jax.Array,
    B_w_down: jax.Array,
    gate_w: jax.Array,
):
    del B_x
    assert A_x.shape == (1, S, D) and A_wqkv.shape == (D, 3 * D) and B_w_gate.shape == (D, FF)
    hbm = pl.BlockSpec(memory_space=pl.ANY)
    out = pl.pallas_call(
        _kernel,
        out_shape=jax.ShapeDtypeStruct((S, D), BF16),
        in_specs=[hbm] * 8,
        out_specs=hbm,
        scratch_shapes=[
            pltpu.VMEM((S, D), BF16),
            pltpu.VMEM((D, D), BF16),
            pltpu.VMEM((D, D), BF16),
            pltpu.VMEM((D, D), BF16),
            pltpu.VMEM((D, D), BF16),
            pltpu.VMEM((D + 16, FF), BF16),
            pltpu.VMEM((D + 16, FF), BF16),
            pltpu.VMEM((FF + 16, D), BF16),
            pltpu.VMEM((8, 128), BF16),
            pltpu.VMEM((8, 128), BF16),
            pltpu.VMEM((D, D), BF16),
            pltpu.VMEM((D, D), BF16),
            pltpu.VMEM((D, S), BF16),
            pltpu.VMEM((S, D), BF16),
            pltpu.VMEM((D, D), BF16),
            pltpu.VMEM((D, D), BF16),
            pltpu.VMEM((D, 128), F32),
            pltpu.VMEM((FF, 128), F32),
            pltpu.VMEM((S, 128), F32),
            pltpu.SemaphoreType.DMA((NUM_COPIES,)),
        ],
        compiler_params=pltpu.CompilerParams(
            vmem_limit_bytes=110 * 1024 * 1024,
            flags={"XLA_TPU_EVENLY_DISTRIBUTE_CRITICAL_NODES": True},
        ),
        name="gated_mix_linear_attn_mod",
    )(A_x.reshape(S, D), A_wqkv, A_wo, B_w_r.reshape(8, 128),
      B_w_gate, B_w_up, B_w_down, gate_w.reshape(8, 128))
    return out.reshape(1, S, D)
```

```python
import jax
import jax.numpy as jnp
import jax.experimental.pallas as pl
import jax.experimental.pallas.tpu as pltpu

F32 = jnp.float32
BF16 = jnp.bfloat16

S = 2048
D = 1024
FF = 3584
DH = 32
PF = 256
PT = 512
GF = 512
MR = 64
MC = 512
X_PARTS = ((0, 256), (256, 512), (512, 640), (640, 2048))
WK_PARTS = ((0, 256), (256, 512), (512, 1024))
OUT_PARTS = ((0, 0, 512), (1, 0, 512), (2, 0, 512), (3, 0, 320), (3, 320, 128), (3, 448, 64))
NUM_COPIES = len(X_PARTS) + len(WK_PARTS) + len(OUT_PARTS) + 8
F32_MAX = 3.4028234663852886e38

NT_DIMS = (((1,), (1,)), ((), ()))
TT_DIMS = (((0,), (1,)), ((), ()))


def _phi(t):
    return jnp.where(t > 0, t + 1.0, jnp.exp(t)) + 1e-6


def _sigmoid(t):
    return 1.0 / (1.0 + jnp.exp(-t))


def _lanes(v, n):
    return v if n == 1 else jnp.concatenate([v] * n, axis=1)


def _fold_lanes(v):
    acc = v[:, 0:128]
    for j in range(1, v.shape[1] // 128):
        acc = acc + v[:, j * 128:(j + 1) * 128]
    return acc


def _as_column(row):
    tiles = [jnp.broadcast_to(row[:, j * 128:(j + 1) * 128], (128, 128)).T
             for j in range(row.shape[1] // 128)]
    return tiles[0] if len(tiles) == 1 else jnp.concatenate(tiles, axis=0)


def _row_vector(v_ref):
    v = v_ref[...].astype(F32)
    return jnp.concatenate([v[j:j + 1, :] for j in range(8)], axis=1)


def _interleave(main, side=(), carry=None):
    pending, done = carry, 0
    for k, piece in enumerate(main):
        epilogue = piece()
        if pending is not None:
            pending()
        pending = epilogue
        upto = (k + 1) * len(side) // len(main)
        for job in side[done:upto]:
            job()
        done = upto
    return pending


def _kernel(x_hbm, wqkv_hbm, wo_hbm, wr_hbm, wg_hbm, wu_hbm, wd_hbm, gw_hbm, out_hbm,
            x_v, wk_v, wq_v, wv_v, wo_v, wg_v, wu_v, wd_v, wr_v, gw_v,
            wkt_v, wqt_v, pk_v, pq_v, g_v, m_v, xcol_v, hcol_v, mix_v, sems):
    copies = {}

    def define(name, src, dst):
        copies[name] = pltpu.make_async_copy(src, dst, sems.at[len(copies)])

    def start(*names):
        for n in names:
            copies[n].start()

    def wait(*names):
        for n in names:
            copies[n].wait()

    for i, (t0, t1) in enumerate(X_PARTS):
        define(("x", i), x_hbm.at[pl.ds(t0, t1 - t0), :], x_v.at[pl.ds(t0, t1 - t0), :])
    for i, (c0, c1) in enumerate(WK_PARTS):
        define(("wk", i), wqkv_hbm.at[:, pl.ds(D + c0, c1 - c0)], wk_v.at[:, pl.ds(c0, c1 - c0)])
    define("wq", wqkv_hbm.at[:, pl.ds(0, D)], wq_v)
    define("wv", wqkv_hbm.at[:, pl.ds(2 * D, D)], wv_v)
    define("wo", wo_hbm, wo_v)
    define("wg", wg_hbm, wg_v.at[pl.ds(0, D), :])
    define("wu", wu_hbm, wu_v.at[pl.ds(0, D), :])
    define("wd", wd_hbm, wd_v.at[pl.ds(0, FF), :])
    define("wr", wr_hbm, wr_v)
    define("gw", gw_hbm, gw_v)

    z_acc = {}

    def key_piece(f0, t0, nt=PT, transposed=True):
        def piece():
            if transposed:
                kt = jax.lax.dot_general(wkt_v[f0:f0 + PF, :], x_v[t0:t0 + nt, :], NT_DIMS,
                                         preferred_element_type=F32)
            else:
                kt = jax.lax.dot_general(wk_v[:, f0:f0 + PF], x_v[t0:t0 + nt, :], TT_DIMS,
                                         preferred_element_type=F32)

            def epilogue():
                pk = _phi(kt)
                pk_v[f0:f0 + PF, t0:t0 + nt] = pk.astype(BF16)
                part = _fold_lanes(pk)
                z_acc[f0] = z_acc[f0] + part if f0 in z_acc else part
            return epilogue
        return piece

    def transpose_job(src_v, dst_v, f0):
        def job():
            dst_v[f0:f0 + PF, :] = src_v[:, f0:f0 + PF].T
        return job

    start(("wk", 0), ("x", 0), ("x", 1), ("wk", 1), ("wk", 2), ("x", 2), ("x", 3),
          "wr", "gw", "wg", "wq", "wv", "wo", "wu", "wd")
    wait(("wk", 0), ("x", 0))
    last = _interleave([key_piece(0, 0, 256, False)])
    wait(("x", 1))
    last = _interleave([key_piece(0, 256, 256, False)], carry=last)
    wait(("wk", 1))
    last = _interleave([key_piece(PF, 0, PT, False)], carry=last)
    wait(("wk", 2), ("x", 2))
    last = _interleave([key_piece(f0, 512, 128, False) for f0 in (0, PF)]
                       + [key_piece(f0, 0, 640, False) for f0 in (2 * PF, 3 * PF)],
                       [transpose_job(wk_v, wkt_v, f0) for f0 in range(0, D, PF)], carry=last)
    wait(("x", 3), "wr", "gw")

    wr_row = _row_vector(wr_v)
    gw_row = _row_vector(gw_v)
    sub = jax.lax.broadcasted_iota(jnp.int32, (8, 1), 0)
    best = [jnp.full((8, 1), -jnp.inf, F32), sub]

    def score_job(t0):
        def job():
            xf = x_v[t0:t0 + 64, :].astype(F32)
            g = _sigmoid(jnp.sum(_fold_lanes(xf * gw_row), axis=1, keepdims=True))
            mix_v[t0:t0 + 64, :] = jnp.broadcast_to(g, (64, 128))
            r = jnp.sum(_fold_lanes(xf * wr_row), axis=1, keepdims=True)
            r = r.astype(BF16).astype(F32)
            key = jnp.where(r != r, -jnp.inf, jnp.maximum(r, -F32_MAX))
            for k in range(0, 64, 8):
                better = key[k:k + 8] > best[0]
                best[0] = jnp.where(better, key[k:k + 8], best[0])
                best[1] = jnp.where(better, sub + (t0 + k), best[1])
        return job

    routed = {}

    def select_job():
        top = jnp.max(best[0], axis=0, keepdims=True)
        token = jnp.min(jnp.where(best[0] == top, best[1], S))
        group = x_v[pl.ds(pl.multiple_of((token // 16) * 16, 16), 16), :].astype(F32)
        hit = jax.lax.broadcasted_iota(jnp.int32, (16, D), 0) == token % 16
        routed["token"] = token
        routed["x"] = jnp.sum(jnp.where(hit, group, 0.0), axis=0, keepdims=True)

    last = _interleave([key_piece(f0, t0, nt) for t0, nt in ((640, 384), (1024, 1024)) for f0 in range(0, D, PF)],
                       [score_job(t0) for t0 in range(0, S, 64)] + [select_job] + [lambda: None] * 8,
                       carry=last)
    token, x_sel = routed["token"], routed["x"]
    weight = _sigmoid(jnp.sum(x_sel * wr_row, axis=1, keepdims=True))

    zero = pl.multiple_of((token // S) * 16, 16)
    acc = {}

    def matvec_job(name, w_v, col_v, r0, c0):
        def job():
            a = acc.get((name, c0))
            for r in range(r0, r0 + MR, 8):
                w = w_v[pl.ds(zero + r, 8), c0:c0 + MC].astype(F32)
                p = w * _lanes(col_v[r:r + 8, :], MC // 128)
                a = p if a is None else a + p
            acc[name, c0] = a
            w_v[w_v.shape[0] - 16:, 0:128] = jnp.concatenate([_fold_lanes(a)] * 2, axis=0).astype(BF16)
        return job

    def matvec_jobs(name, w_v, col_v):
        return [matvec_job(name, w_v, col_v, r0, c0)
                for c0 in range(0, w_v.shape[1], MC) for r0 in range(0, col_v.shape[0], MR)]

    def total(name, c0):
        return jnp.sum(acc[name, c0], axis=0, keepdims=True)

    def token_column_job(c0):
        def job():
            xcol_v[c0:c0 + 128, :] = _as_column(x_sel[:, c0:c0 + 128])
        return job

    def hidden_job(c0):
        def job():
            gate = total("gate", c0)
            hcol_v[c0:c0 + MC, :] = _as_column(gate * _sigmoid(gate) * total("up", c0))
        return job

    def g_piece(f0):
        def piece():
            g = jnp.dot(pk_v[f0:f0 + GF, :], x_v[...], preferred_element_type=F32)

            def epilogue():
                g_v[f0:f0 + GF, :] = g.astype(BF16)
            return epilogue
        return piece

    last = _interleave([g_piece(0)], [token_column_job(c0) for c0 in range(0, D, 128)], carry=last)
    wait("wg", "wq", "wv", "wo")
    last = _interleave([g_piece(f0) for f0 in range(GF, D, GF)],
                       matvec_jobs("gate", wg_v, xcol_v)
                       + [transpose_job(wq_v, wqt_v, f0) for f0 in range(0, D, PF)], carry=last)
    z_col = {f0: jnp.broadcast_to(jnp.sum(z, axis=1, keepdims=True), (PF, 128))
             for f0, z in z_acc.items()}

    def query_piece(f0, t0):
        def piece():
            qt = jax.lax.dot_general(wqt_v[f0:f0 + PF, :], x_v[t0:t0 + PT, :], NT_DIMS,
                                     preferred_element_type=F32)

            def epilogue():
                pq = _phi(qt)
                den = jnp.sum((pq * _lanes(z_col[f0], PT // 128)).reshape(PF // DH, DH, PT),
                              axis=1, keepdims=True) + 1e-6
                pn = pq.reshape(PF // DH, DH, PT) * (1.0 / den)
                pq_v[t0:t0 + PT, f0:f0 + PF] = pn.reshape(PF, PT).astype(BF16).T
            return epilogue
        return piece

    same_head = (jax.lax.broadcasted_iota(jnp.int32, (128, 128), 0) // DH
                 == jax.lax.broadcasted_iota(jnp.int32, (128, 128), 1) // DH)
    kv = {}

    def kv_job(f0):
        def job():
            full = jnp.dot(g_v[f0:f0 + 128, :], wv_v[:, f0:f0 + 128], preferred_element_type=F32)
            kv[f0] = jnp.where(same_head, full, 0.0).astype(BF16)
        return job

    def m_job(f0):
        def job():
            m_v[f0:f0 + 128, :] = jnp.dot(kv[f0], wo_v[f0:f0 + 128, :],
                                          preferred_element_type=F32).astype(BF16)
        return job

    late = 5 * 128
    last = _interleave([query_piece(f0, t0) for t0 in range(0, S, PT) for f0 in range(0, D, PF)],
                       [job for f0 in range(0, D, 128)
                        for job in [kv_job(f0)] + ([m_job(f0)] if f0 < late else [])], carry=last)
    last = _interleave([m_job(f0) for f0 in range(late, D, 128)], carry=last)
    assert last is None

    wait("wu", "wd")
    tiles = S // PT

    def out_piece(i):
        def piece():
            k, r0, nr = OUT_PARTS[i]
            t0 = pl.multiple_of(((token // PT + 1 + k) % tiles) * PT + r0, 64)
            rows = pl.ds(t0, nr)
            a = jnp.dot(pq_v[rows, :], m_v[...], preferred_element_type=F32)

            def epilogue():
                xf = x_v[rows, :].astype(F32)
                g = mix_v[rows, :]
                upd = xf * 0.0
                if k == tiles - 1:
                    y = jnp.concatenate([total("down", c0) for c0 in range(0, D, MC)], axis=1) * weight
                    is_token = jax.lax.broadcasted_iota(jnp.int32, (nr, D), 0) + t0 == token
                    upd = upd + jnp.where(is_token, y, 0.0)
                mixed = _lanes(g, D // 128) * a + _lanes(1.0 - g, D // 128) * (xf + upd)
                x_v[rows, :] = mixed.astype(BF16)
                define(("out", i), x_v.at[rows, :], out_hbm.at[rows, :])
                start(("out", i))
            return epilogue
        return piece

    last = _interleave([out_piece(i) for i in range(len(OUT_PARTS) - 2)],
                       matvec_jobs("up", wu_v, xcol_v) + [hidden_job(c0) for c0 in range(0, FF, MC)]
                       + matvec_jobs("down", wd_v, hcol_v))
    last = _interleave([out_piece(i) for i in range(len(OUT_PARTS) - 2, len(OUT_PARTS))], carry=last)
    last()
    wait(*[("out", i) for i in range(len(OUT_PARTS))])


@jax.jit
def pallas_gated_mix__linear_attn_block__moe_arch_mod__prompt_kernel(
    A_x: jax.Array,
    A_wqkv: jax.Array,
    A_wo: jax.Array,
    B_x: jax.Array,
    B_w_r: jax.Array,
    B_w_gate: jax.Array,
    B_w_up: jax.Array,
    B_w_down: jax.Array,
    gate_w: jax.Array,
):
    del B_x
    assert A_x.shape == (1, S, D) and A_wqkv.shape == (D, 3 * D) and B_w_gate.shape == (D, FF)
    hbm = pl.BlockSpec(memory_space=pl.ANY)
    out = pl.pallas_call(
        _kernel,
        out_shape=jax.ShapeDtypeStruct((S, D), BF16),
        in_specs=[hbm] * 8,
        out_specs=hbm,
        scratch_shapes=[
            pltpu.VMEM((S, D), BF16),
            pltpu.VMEM((D, D), BF16),
            pltpu.VMEM((D, D), BF16),
            pltpu.VMEM((D, D), BF16),
            pltpu.VMEM((D, D), BF16),
            pltpu.VMEM((D + 16, FF), BF16),
            pltpu.VMEM((D + 16, FF), BF16),
            pltpu.VMEM((FF + 16, D), BF16),
            pltpu.VMEM((8, 128), BF16),
            pltpu.VMEM((8, 128), BF16),
            pltpu.VMEM((D, D), BF16),
            pltpu.VMEM((D, D), BF16),
            pltpu.VMEM((D, S), BF16),
            pltpu.VMEM((S, D), BF16),
            pltpu.VMEM((D, D), BF16),
            pltpu.VMEM((D, D), BF16),
            pltpu.VMEM((D, 128), F32),
            pltpu.VMEM((FF, 128), F32),
            pltpu.VMEM((S, 128), F32),
            pltpu.SemaphoreType.DMA((NUM_COPIES,)),
        ],
        compiler_params=pltpu.CompilerParams(
            vmem_limit_bytes=110 * 1024 * 1024,
            flags={"XLA_TPU_EVENLY_DISTRIBUTE_CRITICAL_NODES": True},
        ),
        name="gated_mix_linear_attn_mod",
    )(A_x.reshape(S, D), A_wqkv, A_wo, B_w_r.reshape(8, 128),
      B_w_gate, B_w_up, B_w_down, gate_w.reshape(8, 128))
    return out.reshape(1, S, D)
```
